```python
import os as _os
_os.environ.setdefault("JAX_PLATFORMS", "cpu")
import jax
import jax.numpy as jnp

def _softmax(x, axis=-1):
    return jax.nn.softmax(x, axis=axis)
def _gelu(x):
    return jax.nn.gelu(x, approximate=True)
def _silu(x):
    return jax.nn.silu(x)
def _sigmoid(x):
    return jax.nn.sigmoid(x)
def _layernorm(x, axis=-1, eps=1e-5):
    m = jnp.mean(x, axis=axis, keepdims=True)
    v = jnp.var(x, axis=axis, keepdims=True)
    return (x - m) / jnp.sqrt(v + eps)
def _scatter_add(tgt, idx, src, axis=0):
    return tgt.at[idx].add(src)
def _segment_sum(src, seg, n):
    return jax.ops.segment_sum(src, seg, n)
class _Rng:
    def __init__(self, key):
        self._k = key
    def _next(self):
        self._k, sub = jax.random.split(self._k)
        return sub
    def normal(self, shape):
        return jax.random.normal(self._next(), shape, dtype=jnp.bfloat16)
    def randint(self, lo, hi, shape):
        return jax.random.randint(self._next(), shape, lo, hi, dtype=jnp.int32)
    def uniform(self, shape, lo=0.0, hi=1.0):
        return jax.random.uniform(self._next(), shape, jnp.bfloat16, lo, hi)
    def permutation(self, n):
        return jax.random.permutation(self._next(), n)


kernel_name = 'interleave_layers__sliding_block_cached__mixer_channel_mlp__decode'

def setup_inputs():
    _rng = _Rng(jax.random.key(int.from_bytes(__import__("os").urandom(4), "little")))
    _w = (lambda a: (lambda t: t.astype(jnp.bfloat16) if jnp.issubdtype(t.dtype, jnp.floating) else t)(jnp.asarray(a)))
    def _A_setup():
        B, Sq, D = 8, 1, 1024
        Hq, Hkv, Sk, Dh = 32, 4, 4096, 128
        assert Hq % Hkv == 0, (Hq, Hkv)
        return {
            "x": _w((lambda *s: _rng.normal(s) * 0.05)(B, Sq, D)),
            "k_cache": _w((lambda *s: _rng.normal(s) * 1.6)(B, Hkv, Sk, Dh)),
            "v_cache": _w((lambda *s: _rng.normal(s) * 0.8)(B, Hkv, Sk, Dh)),
            "wq": _w((lambda *s: _rng.normal(s) * 1.6)(D, Hq * Dh) * (D ** -0.5)),
            "wo": _w((lambda *s: _rng.normal(s) * 0.8)(Hq * Dh, D) * ((Hq * Dh) ** -0.5)),
        }
    _A_in = _A_setup()

    def _B_setup():
        B, S, D, F = 8, 1, 1024, 3584
        return {
            "x": _w((lambda *s: _rng.normal(s) * 0.05)(B, S, D)),
            "w1": _w((lambda *s: _rng.normal(s) * 0.4)(D, F) * (D ** -0.5)),
            "b1": _w((lambda *s: _rng.normal(s) * 0.4)(F)),
            "w2": _w((lambda *s: _rng.normal(s) * 0.4)(F, D) * (F ** -0.5)),
            "b2": _w((lambda *s: _rng.normal(s) * 0.1)(D)),
        }
    _B_in = _B_setup()

    return {
        "A_x": _A_in["x"],
        "A_k_cache": _A_in["k_cache"],
        "A_v_cache": _A_in["v_cache"],
        "A_wq": _A_in["wq"],
        "A_wo": _A_in["wo"],
        "B_x": _B_in["x"],
        "B_w1": _B_in["w1"],
        "B_b1": _B_in["b1"],
        "B_w2": _B_in["w2"],
        "B_b2": _B_in["b2"],
    }

def reference(A_x, A_k_cache, A_v_cache, A_wq, A_wo, B_x, B_w1, B_b1, B_w2, B_b2):
    def _A_ref(x, k_cache, v_cache, wq, wo):
        B, Sq, D = x.shape
        Hq, Dh = 32, 128
        Hkv, Sk = k_cache.shape[1], k_cache.shape[2]
        W = min(4096, max(256, Sk // 4))
        rep = Hq // Hkv
        q = (lambda x, *d: x.transpose(*d))((x @ wq).reshape(B, Sq, Hq, Dh), 0, 2, 1, 3)
        k = jnp.repeat(k_cache[:, :, Sk - W:, :], rep, axis=1)
        v = jnp.repeat(v_cache[:, :, Sk - W:, :], rep, axis=1)
        scores = jnp.einsum("bhqd,bhkd->bhqk", q, k) * (Dh ** -0.5)
        p = _softmax(scores, axis=-1)
        o = jnp.einsum("bhqk,bhkd->bhqd", p, v)
        return (lambda x, *d: x.transpose(*d))(o, 0, 2, 1, 3).reshape(B, Sq, Hq * Dh) @ wo

    def _B_ref(x, w1, b1, w2, b2):
        y = _layernorm(x, axis=-1)
        h = _gelu(jnp.einsum("bsd,df->bsf", y, w1) + b1)
        return jnp.einsum("bsf,fd->bsd", h, w2) + b2

    x = A_x
    x = x + _A_ref(_layernorm(x, axis=-1), A_k_cache, A_v_cache, A_wq, A_wo)
    x = x + _B_ref(_layernorm(x, axis=-1), B_w1, B_b1, B_w2, B_b2)
    x = x + _A_ref(_layernorm(x, axis=-1), A_k_cache, A_v_cache, A_wq, A_wo)
    x = x + _B_ref(_layernorm(x, axis=-1), B_w1, B_b1, B_w2, B_b2)
    return x
```

```python
import functools
import math

import jax
import jax.numpy as jnp
from jax import lax
import jax.experimental.pallas as pl
import jax.experimental.pallas.tpu as pltpu

_BF = jnp.bfloat16
_F32 = jnp.float32
_EPS = 1e-5
_T = 128
_NB = 4 * _T
_HQ = 32


def _mm(a, b):
    return jnp.dot(a, b, preferred_element_type=_F32)


def _ln_stats(x):
    m = jnp.mean(x, axis=-1, keepdims=True)
    d = x - m
    v = jnp.mean(d * d, axis=-1, keepdims=True)
    return m, d, lax.rsqrt(v + _EPS)


def _gelu(x):
    c = math.sqrt(2.0 / math.pi)
    return x * (0.5 * (1.0 + jnp.tanh(c * (x + 0.044715 * (x * x * x)))))


def _swap8(vs):
    row = lax.broadcasted_iota(jnp.int32, (8, _T), 0)
    vs = list(vs)
    for s in (4, 2, 1):
        hi = (row & s) != 0
        out = [None] * 8
        for i in range(8):
            if i & s:
                continue
            a, b = vs[i], vs[i + s]
            out[i] = jnp.where(hi, pltpu.roll(b, s, 0), a)
            out[i + s] = jnp.where(hi, b, pltpu.roll(a, 8 - s, 0))
        vs = out
    return vs


def _kernel(x_h, k_h, v_h, wq_h, wo_h, w1_h, b1_h, w2_h, b2_h, o_h,
            x_s, k_s, kt_s, v_s, wq_s, wo_s, w1_s, b1_s, w2_s, b2_s,
            q_s, cq_s, c1_s, p_s, l_s, a_s, h_s, r_s, out_s, sems,
            *, w2_rows):
    nb_, d_model = x_s.shape
    hkv, win, dh = k_s.shape[1], k_s.shape[2], k_s.shape[3]
    rep = _HQ // hkv
    d_ff = w1_s.shape[1]
    sk = k_h.shape[2]
    kd, kf = d_model // _T, d_ff // _T
    sm_c = dh ** -0.5 * math.log2(math.e)
    r_tail = w2_rows[-1]

    copies = [
        (wq_h, wq_s), (x_h, x_s), (b1_h, b1_s), (b2_h, b2_s),
        (k_h.at[:, :, pl.ds(sk - win, win)], k_s),
        (v_h.at[:, :, pl.ds(sk - win, win)], v_s),
        (wo_h, wo_s), (w1_h, w1_s),
    ]
    for r0, r1 in zip(w2_rows[:-1], w2_rows[1:]):
        copies.append((w2_h.at[pl.ds(r0, r1 - r0)], w2_s.at[pl.ds(r0, r1 - r0)]))
    dmas = [pltpu.make_async_copy(a, b, sems.at[i]) for i, (a, b) in enumerate(copies)]
    n_fix = len(dmas)

    def tail_dma(c):
        idx = (pl.ds(r_tail, d_ff - r_tail), pl.ds(pl.multiple_of(c * _T, _T), _T))
        return pltpu.make_async_copy(w2_h.at[idx], w2_s.at[idx], sems.at[n_fix + c])

    for d in dmas:
        d.start()
    for c in range(kd):
        tail_dma(c).start()
    d_wq, d_x, d_b1, d_b2, d_k, d_v, d_wo, d_w1 = dmas[:8]

    def tile(v, i):
        return v[:, i * _T:(i + 1) * _T]

    def proj(lhs, w_ref, cols):
        acc = None
        for k in range(lhs.shape[1] // _T):
            y = _mm(tile(lhs, k), w_ref[k * _T:(k + 1) * _T, cols])
            acc = y if acc is None else acc + y
        return acc

    ones = jnp.ones((nb_, d_model), _F32)

    d_x.wait()
    x0 = x_s[...].astype(_F32)
    _, d0, r0_ = _ln_stats(x0)
    lhs = jnp.concatenate([d0 * r0_, ones], axis=0).astype(_BF)
    d_wq.wait()

    @pl.loop(0, hkv)
    def _(j):
        qs = []
        for n in range(rep * dh // _NB):
            cols = pl.ds(pl.multiple_of(j * (rep * dh) + n * _NB, _NB), _NB)
            y = proj(lhs, wq_s, cols)
            cq_s[:, cols] = y[nb_:]
            qs += [tile(y[:nb_], i) for i in range(_NB // _T)]
        for b, qb in enumerate(_swap8(qs)):
            q_s[j * nb_ + b] = qb

    d_k.wait()

    @pl.loop(0, hkv * nb_)
    def _(g):
        kt = k_s[g % nb_, g // nb_].T
        kt_s[g] = kt
        s = _mm(q_s[g].astype(_BF), kt)
        p = jnp.exp2((s - jnp.max(s, axis=-1, keepdims=True)) * sm_c)
        l_s[g] = jnp.broadcast_to(1.0 / jnp.sum(p, axis=-1, keepdims=True), (rep, dh))
        p_s[g] = p

    d_v.wait()

    @pl.loop(0, hkv)
    def _(j):
        os_ = []
        for b in range(nb_):
            g = j * nb_ + b
            os_.append(_mm(p_s[g].astype(_BF), v_s[b, j]) * l_s[g])
        for r, o in enumerate(_swap8(os_)):
            a_s[j * rep + r] = o

    d_wo.wait()

    def wo_body(j, acc):
        for r in range(rep):
            hd = j * rep + r
            rows = pl.ds(pl.multiple_of(hd * dh, dh), dh)
            acc = acc + _mm(a_s[hd].astype(_BF), wo_s[rows, :])
        return acc

    x1 = lax.fori_loop(0, hkv, wo_body, x0)

    _, d1, r1_ = _ln_stats(x1)
    _, d1, r1_ = _ln_stats(d1 * r1_)
    lhs = jnp.concatenate([d1 * r1_, ones], axis=0).astype(_BF)
    d_b1.wait()
    d_b2.wait()
    b2 = b2_s[...].astype(_F32).reshape(1, d_model)
    c1_s[0] = jnp.broadcast_to(b1_s[...].astype(_F32).reshape(1, d_ff), (nb_, d_ff))
    d_w1.wait()

    @pl.loop(0, d_ff // _NB)
    def _(n):
        cols = pl.ds(pl.multiple_of(n * _NB, _NB), _NB)
        y = proj(lhs, w1_s, cols)
        c1_s[1, :, cols] = y[nb_:]
        h_s[:, cols] = _gelu(y[:nb_] + c1_s[0, :, cols])

    acc = x1 + b2
    for i, (r0, r1) in enumerate(zip(w2_rows[:-1], w2_rows[1:])):
        dmas[8 + i].wait()

        def w2_body(n, acc):
            for k in range(_NB // _T):
                ks = pl.ds(pl.multiple_of(n * _NB + k * _T, _T), _T)
                acc = acc + _mm(h_s[:, ks].astype(_BF), w2_s[ks, :])
            return acc

        acc = lax.fori_loop(r0 // _NB, r1 // _NB, w2_body, acc)
    r_s[...] = acc
    h_tail = h_s[:, r_tail:].astype(_BF)

    def finish_cols(c):
        tail_dma(c).wait()
        cols = pl.ds(pl.multiple_of(c * _T, _T), _T)
        xc = r_s[:, cols] + proj(h_tail, w2_s.at[r_tail:], cols)
        r_s[:, cols] = xc
        return xc.astype(_BF), cols

    q_s[...] = jnp.zeros(q_s.shape, _F32)

    @pl.loop(0, kd - 1)
    def _(c):
        xc, rows = finish_cols(c)
        for n in range(_HQ * dh // _NB):
            y = _mm(xc, wq_s[rows, n * _NB:(n + 1) * _NB])
            for i in range(_NB // _T):
                q_s[n * (_NB // _T) + i] += tile(y, i)

    xc, rows = finish_cols(kd - 1)
    x2 = r_s[...]
    m, _, rstd = _ln_stats(x2.astype(_BF).astype(_F32))
    qg = []
    for j in range(hkv):
        qs = []
        for n in range(j * rep * dh // _NB, (j + 1) * rep * dh // _NB):
            y = _mm(xc, wq_s[rows, n * _NB:(n + 1) * _NB])
            for i in range(_NB // _T):
                hd = n * (_NB // _T) + i
                qs.append((q_s[hd] + tile(y, i) - m * cq_s[:, hd * dh:(hd + 1) * dh]) * rstd)
        qs = _swap8(qs)
        for b in range(0, nb_, 2):
            qg.append(jnp.concatenate(qs[b:b + 2], axis=0).astype(_BF))

    def qk(i):
        ps, ls = [], []
        for u in range(2):
            s = _mm(qg[i], kt_s[2 * i + u])[u * rep:(u + 1) * rep]
            p = jnp.exp2((s - jnp.max(s, axis=-1, keepdims=True)) * sm_c)
            ls.append(1.0 / jnp.sum(p, axis=-1, keepdims=True))
            ps.append(p)
        return jnp.concatenate(ps, axis=0).astype(_BF), ls

    def pv(i, p, ls):
        j, b = divmod(2 * i, nb_)
        return [_mm(p, v_s[b + u, j])[u * rep:(u + 1) * rep] * ls[u] for u in range(2)]

    n_pair = hkv * nb_ // 2
    ahead = 2
    pend, os_, heads = {}, [], []
    for i in range(n_pair + ahead):
        if i < n_pair:
            pend[i] = qk(i)
        if i >= ahead:
            os_ += pv(i - ahead, *pend.pop(i - ahead))
            if len(os_) == nb_:
                heads += [o.astype(_BF) for o in _swap8(os_)]
                os_ = []

    x3 = []
    for n in range(d_model // _NB):
        acc = x2[:, n * _NB:(n + 1) * _NB]
        for hd in range(_HQ):
            acc = acc + _mm(heads[hd], wo_s[hd * dh:(hd + 1) * dh, n * _NB:(n + 1) * _NB])
        x3.append(acc)
    x3b = [v.astype(_BF) for v in x3]
    x3 = jnp.concatenate(x3, axis=1)

    m1, d3, r3 = _ln_stats(jnp.concatenate(x3b, axis=1).astype(_F32))
    m2, _, r4 = _ln_stats(d3 * r3)
    sa = r3 * r4
    sb = (m1 * r3 + m2) * r4

    def w1_part(n, half, acc):
        for k in range(_NB // _T):
            kk = half * (_NB // _T) + k
            y = _mm(tile(x3b[half], k), w1_s[kk * _T:(kk + 1) * _T, n * _NB:(n + 1) * _NB])
            acc = y if acc is None else acc + y
        return acc

    lead = 2
    part = [w1_part(n, 0, None) for n in range(lead)]
    hs = []
    for n in range(d_ff // _NB):
        y = w1_part(n, 1, part[n] if n < lead else w1_part(n, 0, None))
        cols = slice(n * _NB, (n + 1) * _NB)
        hs.append(_gelu(y * sa - sb * c1_s[1, :, cols] + c1_s[0, :, cols]).astype(_BF))

    acc = x3 + b2
    for k in range(kf):
        acc = acc + _mm(tile(hs[k // (_NB // _T)], k % (_NB // _T)), w2_s[k * _T:(k + 1) * _T, :])
    out_s[...] = acc.astype(out_s.dtype)
    pltpu.sync_copy(out_s, o_h)


@jax.jit
def pallas_interleave_layers__sliding_block_cached__mixer_channel_mlp__decode_kernel(
    A_x: jax.Array,
    A_k_cache: jax.Array,
    A_v_cache: jax.Array,
    A_wq: jax.Array,
    A_wo: jax.Array,
    B_x: jax.Array,
    B_w1: jax.Array,
    B_b1: jax.Array,
    B_w2: jax.Array,
    B_b2: jax.Array,
):
    del B_x
    nb_, sq, d_model = A_x.shape
    _, hkv, sk, dh = A_k_cache.shape
    d_ff = B_w1.shape[1]
    win = min(4096, max(256, sk // 4))
    rep = _HQ // hkv
    assert (nb_, sq, rep, dh) == (8, 1, 8, _T)
    w2_rows = (0, 1536, 2560, 3072)
    n_sem = 8 + len(w2_rows) - 1 + d_model // _T

    hbm = pl.BlockSpec(memory_space=pltpu.HBM)
    vmem = pltpu.VMEM
    out = pl.pallas_call(
        functools.partial(_kernel, w2_rows=w2_rows),
        out_shape=jax.ShapeDtypeStruct((nb_, d_model), A_x.dtype),
        in_specs=[hbm] * 9,
        out_specs=hbm,
        scratch_shapes=[
            vmem((nb_, d_model), A_x.dtype),
            vmem((nb_, hkv, win, dh), _BF),
            vmem((nb_ * hkv, dh, win), _BF),
            vmem((nb_, hkv, win, dh), _BF),
            vmem(A_wq.shape, _BF),
            vmem(A_wo.shape, _BF),
            vmem(B_w1.shape, _BF),
            vmem(B_b1.shape, B_b1.dtype),
            vmem(B_w2.shape, _BF),
            vmem(B_b2.shape, B_b2.dtype),
            vmem((_HQ, nb_, dh), _F32),
            vmem((nb_, _HQ * dh), _F32),
            vmem((2, nb_, d_ff), _F32),
            vmem((nb_ * hkv, rep, win), _F32),
            vmem((nb_ * hkv, rep, dh), _F32),
            vmem((_HQ, nb_, dh), _F32),
            vmem((nb_, d_ff), _F32),
            vmem((nb_, d_model), _F32),
            vmem((nb_, d_model), A_x.dtype),
            pltpu.SemaphoreType.DMA((n_sem,)),
        ],
        compiler_params=pltpu.CompilerParams(vmem_limit_bytes=100 * 1024 * 1024),
    )(A_x.reshape(nb_, d_model), A_k_cache, A_v_cache, A_wq, A_wo, B_w1, B_b1, B_w2, B_b2)
    return out.reshape(nb_, sq, d_model)
```

```python
import math

import jax
import jax.numpy as jnp
from jax import lax
import jax.experimental.pallas as pl
import jax.experimental.pallas.tpu as pltpu

_BF = jnp.bfloat16
_F32 = jnp.float32
_EPS = 1e-5
_T = 128
_NB = 4 * _T
_HQ = 32
_W2_MID, _W2_TAIL = 1664, 2560
_W2_LEFT = 4
_SIDE = 176
_PRIO = 1
_HOLD = 2


def _mm(a, b):
    return jnp.dot(a, b, preferred_element_type=_F32)


def _ln_stats(x):
    m = jnp.mean(x, axis=-1, keepdims=True)
    d = x - m
    v = jnp.mean(d * d, axis=-1, keepdims=True)
    return m, d, lax.rsqrt(v + _EPS)


def _gelu(x):
    c = math.sqrt(2.0 / math.pi)
    return x * (0.5 * (1.0 + jnp.tanh(c * (x + 0.044715 * (x * x * x)))))


def _swap8(vs):
    row = lax.broadcasted_iota(jnp.int32, (8, _T), 0)
    vs = list(vs)
    for s in (4, 2, 1):
        hi = (row & s) != 0
        out = [None] * 8
        for i in range(8):
            if i & s:
                continue
            a, b = vs[i], vs[i + s]
            out[i] = jnp.where(hi, pltpu.roll(b, s, 0), a)
            out[i + s] = jnp.where(hi, b, pltpu.roll(a, 8 - s, 0))
        vs = out
    return vs


def _kernel(x_h, k_h, v_h, wq_h, wo_h, w1_h, b1_h, w2_h, b2_h, o_h,
            x_s, k_s, kt_s, v_s, wq_s, wo_s, w1_s, b1_s, w2_s, w2t_s, b2_s,
            q_s, cq_s, c1_s, p_s, l_s, a_s, h_s, r_s, out_s, side0, side1, sems, side_sems):
    nb_, d_model = x_s.shape
    hkv, win, dh = k_s.shape[1], k_s.shape[2], k_s.shape[3]
    rep = _HQ // hkv
    d_ff = w1_s.shape[1]
    sk = k_h.shape[2]
    kd, kf = d_model // _T, d_ff // _T
    sm_c = dh ** -0.5 * math.log2(math.e)
    r_mid, r_tail, c_left = _W2_MID, _W2_TAIL, _W2_LEFT * _T
    r_side = r_mid - 4 * _SIDE

    bands = [(0, r_side, 0, d_model), (r_mid, r_tail, 0, c_left),
             (r_tail, d_ff, 0, c_left), (r_mid, r_tail, c_left, d_model)]
    copies = [
        (wq_h, wq_s), (x_h, x_s), (b1_h, b1_s), (b2_h, b2_s),
        (k_h.at[:, :, pl.ds(sk - win, win)], k_s),
        (v_h.at[:, :, pl.ds(sk - win, win)], v_s),
        (wo_h, wo_s), (w1_h, w1_s),
    ] + [(w2_h.at[r0:r1, c0:c1], w2_s.at[r0:r1, c0:c1]) for r0, r1, c0, c1 in bands]
    dmas = [pltpu.make_async_copy(a, b, sems.at[i]) for i, (a, b) in enumerate(copies)]
    n_fix = len(dmas) - _W2_LEFT

    def tail_dma(c):
        idx = (pl.ds(r_tail, d_ff - r_tail), pl.ds(c * _T, _T))
        return pltpu.make_async_copy(w2_h.at[idx], w2t_s.at[c - _W2_LEFT], sems.at[n_fix + c])

    def side_in(i):
        return pltpu.make_async_copy(
            w2_h.at[pl.ds(r_side + i * _SIDE, _SIDE)], (side0, side1)[i % 2], side_sems.at[i % 2])

    def side_out(i):
        return pltpu.make_async_copy(
            (side0, side1)[i % 2], w2_s.at[pl.ds(r_side + i * _SIDE, _SIDE)], side_sems.at[i % 2])

    def side_forward(i):
        side_in(i).wait()
        side_out(i).start(priority=_PRIO)

    def side_refill(i):
        side_out(i - 2).wait()
        side_in(i).start(priority=_PRIO)

    dmas[0].start()
    side_in(0).start(priority=_PRIO)
    side_in(1).start(priority=_PRIO)
    for d in dmas[1:]:
        d.start()
    for c in range(_W2_LEFT, kd):
        tail_dma(c).start()
    d_wq, d_x, d_b1, d_b2, d_k, d_v, d_wo, d_w1 = dmas[:8]

    def tile(v, i):
        return v[:, i * _T:(i + 1) * _T]

    def proj(lhs, w_ref, cols):
        acc = None
        for k in range(lhs.shape[1] // _T):
            y = _mm(tile(lhs, k), w_ref[k * _T:(k + 1) * _T, cols])
            acc = y if acc is None else acc + y
        return acc

    ones = jnp.ones((nb_, d_model), _F32)

    side_forward(0)
    d_x.wait()
    x0 = x_s[...].astype(_F32)
    _, d0, r0_ = _ln_stats(x0)
    lhs = jnp.concatenate([d0 * r0_, ones], axis=0).astype(_BF)
    d_wq.wait()

    @pl.loop(0, hkv)
    def _(j):
        qs = []
        for n in range(rep * dh // _NB):
            cols = pl.ds(pl.multiple_of(j * (rep * dh) + n * _NB, _NB), _NB)
            y = proj(lhs, wq_s, cols)
            cq_s[:, cols] = y[nb_:]
            qs += [tile(y[:nb_], i) for i in range(_NB // _T)]
        for b, qb in enumerate(_swap8(qs)):
            q_s[j * nb_ + b] = qb

    side_forward(1)
    d_k.wait()

    @pl.loop(0, hkv * nb_)
    def _(g):
        pl.when(g == 8)(lambda: side_refill(2))
        pl.when(g == 22)(lambda: side_refill(3))
        kt = k_s[g % nb_, g // nb_].T
        kt_s[g] = kt
        s = _mm(q_s[g].astype(_BF), kt)
        p = jnp.exp2((s - jnp.max(s, axis=-1, keepdims=True)) * sm_c)
        l_s[g] = jnp.broadcast_to(1.0 / jnp.sum(p, axis=-1, keepdims=True), (rep, dh))
        p_s[g] = p

    d_v.wait()

    @pl.loop(0, hkv)
    def _(j):
        os_ = []
        for b in range(nb_):
            g = j * nb_ + b
            os_.append(_mm(p_s[g].astype(_BF), v_s[b, j]) * l_s[g])
        for r, o in enumerate(_swap8(os_)):
            a_s[j * rep + r] = o

    side_forward(2)
    d_wo.wait()

    def wo_body(j, acc):
        for r in range(rep):
            hd = j * rep + r
            rows = pl.ds(pl.multiple_of(hd * dh, dh), dh)
            acc = acc + _mm(a_s[hd].astype(_BF), wo_s[rows, :])
        return acc

    x1 = lax.fori_loop(0, hkv, wo_body, x0)

    _, d1, r1_ = _ln_stats(x1)
    _, d1, r1_ = _ln_stats(d1 * r1_)
    lhs = jnp.concatenate([d1 * r1_, ones], axis=0).astype(_BF)
    d_b1.wait()
    d_b2.wait()
    b2 = b2_s[...].astype(_F32).reshape(1, d_model)
    c1_s[0] = jnp.broadcast_to(b1_s[...].astype(_F32).reshape(1, d_ff), (nb_, d_ff))
    side_forward(3)
    d_w1.wait()

    @pl.loop(0, d_ff // _NB)
    def _(n):
        cols = pl.ds(pl.multiple_of(n * _NB, _NB), _NB)
        y = proj(lhs, w1_s, cols)
        c1_s[1, :, cols] = y[nb_:]
        h_s[:, cols] = _gelu(y[:nb_] + c1_s[0, :, cols])

    r_s[...] = x1 + b2

    def w2_part(r0, r1, c0, c1):
        step = _NB if (r1 - r0) % _NB == 0 else r1 - r0

        def body(n, acc):
            for k in range(step // _T):
                ks = pl.ds(pl.multiple_of(r0 + n * step + k * _T, _T), _T)
                acc = acc + _mm(h_s[:, ks].astype(_BF), w2_s[ks, c0:c1])
            return acc

        acc = r_s[:, c0:c1]
        if step == r1 - r0:
            acc = body(0, acc)
        else:
            acc = lax.fori_loop(0, (r1 - r0) // step, body, acc)
        r_s[:, c0:c1] = acc

    q_raw = [None] * _HQ

    n_q = _HQ * dh // _NB

    def q_update(xc, c, blocks):
        for n in blocks:
            y = _mm(xc, wq_s[c * _T:(c + 1) * _T, n * _NB:(n + 1) * _NB])
            for i in range(_NB // _T):
                hd = n * (_NB // _T) + i
                q_raw[hd] = tile(y, i) if q_raw[hd] is None else q_raw[hd] + tile(y, i)

    def w2_band(i):
        dmas[8 + i].wait()
        w2_part(*bands[i])

    r_last = (r_mid - _SIDE) // _T * _T
    dmas[8].wait()
    side_out(2).wait()
    w2_part(0, r_last // _NB * _NB, 0, d_model)
    w2_part(r_last // _NB * _NB, r_last, 0, d_model)
    w2_band(1)
    side_out(3).wait()
    w2_part(r_last, r_mid, 0, d_model)
    w2_band(2)

    x2b = [r_s[:, c * _T:(c + 1) * _T].astype(_BF) for c in range(_W2_LEFT)]
    for c in range(_W2_LEFT):
        q_update(x2b[c], c, range(n_q - (_HOLD if c == _W2_LEFT - 1 else 0)))
    w2_band(3)
    h_tail = h_s[:, r_tail:].astype(_BF)
    for c in range(_W2_LEFT, kd):
        if c == kd - 1:
            seen = jnp.concatenate(x2b, axis=1).astype(_F32)
            m_seen, d_seen, _ = _ln_stats(seen)
            ss_seen = jnp.sum(d_seen * d_seen, axis=-1, keepdims=True)
        tail_dma(c).wait()
        cols = slice(c * _T, (c + 1) * _T)
        xc = r_s[:, cols] + proj(h_tail, w2t_s.at[c - _W2_LEFT], slice(None))
        r_s[:, cols] = xc
        x2b.append(xc.astype(_BF))
        q_update(x2b[c - 1], c - 1, range(n_q - _HOLD, n_q))
        q_update(x2b[c], c, range(n_q - (_HOLD if c < kd - 1 else 0)))

    x2 = r_s[...]
    e = x2b[-1].astype(_F32) - m_seen
    shift = jnp.sum(e, axis=-1, keepdims=True) * (1.0 / d_model)
    var = (ss_seen + jnp.sum(e * e, axis=-1, keepdims=True)) * (1.0 / d_model) - shift * shift
    m, rstd = m_seen + shift, lax.rsqrt(var + _EPS)
    qg = []
    for j in range(hkv):
        qs = _swap8([(q_raw[hd] - m * cq_s[:, hd * dh:(hd + 1) * dh]) * rstd
                     for hd in range(j * rep, (j + 1) * rep)])
        for b in range(0, nb_, 2):
            qg.append(jnp.concatenate(qs[b:b + 2], axis=0).astype(_BF))

    def qk(i):
        ps, ls = [], []
        for u in range(2):
            s = _mm(qg[i], kt_s[2 * i + u])[u * rep:(u + 1) * rep]
            p = jnp.exp2((s - jnp.max(s, axis=-1, keepdims=True)) * sm_c)
            ls.append(1.0 / jnp.sum(p, axis=-1, keepdims=True))
            ps.append(p)
        return jnp.concatenate(ps, axis=0).astype(_BF), ls

    def pv(i, p, ls):
        j, b = divmod(2 * i, nb_)
        return [_mm(p, v_s[b + u, j])[u * rep:(u + 1) * rep] * ls[u] for u in range(2)]

    n_pair = hkv * nb_ // 2
    ahead = 2
    pend, os_, heads = {}, [], []
    for i in range(n_pair + ahead):
        if i < n_pair:
            pend[i] = qk(i)
        if i >= ahead:
            os_ += pv(i - ahead, *pend.pop(i - ahead))
            if len(os_) == nb_:
                heads += [o.astype(_BF) for o in _swap8(os_)]
                os_ = []

    x3 = []
    for n in range(d_model // _NB):
        acc = x2[:, n * _NB:(n + 1) * _NB]
        for hd in range(_HQ):
            acc = acc + _mm(heads[hd], wo_s[hd * dh:(hd + 1) * dh, n * _NB:(n + 1) * _NB])
        x3.append(acc)
    x3b = [v.astype(_BF) for v in x3]
    x3 = jnp.concatenate(x3, axis=1)

    m1, d3, r3 = _ln_stats(jnp.concatenate(x3b, axis=1).astype(_F32))
    m2, _, r4 = _ln_stats(d3 * r3)
    sa = r3 * r4
    sb = (m1 * r3 + m2) * r4

    def w1_part(n, half, acc):
        for k in range(_NB // _T):
            kk = half * (_NB // _T) + k
            y = _mm(tile(x3b[half], k), w1_s[kk * _T:(kk + 1) * _T, n * _NB:(n + 1) * _NB])
            acc = y if acc is None else acc + y
        return acc

    lead = 2
    part = [w1_part(n, 0, None) for n in range(lead)]
    hs = []
    for n in range(d_ff // _NB):
        y = w1_part(n, 1, part[n] if n < lead else w1_part(n, 0, None))
        cols = slice(n * _NB, (n + 1) * _NB)
        hs.append(_gelu(y * sa - sb * c1_s[1, :, cols] + c1_s[0, :, cols]).astype(_BF))

    acc = x3 + b2
    for k in range(kf):
        rows = slice(k * _T, (k + 1) * _T)
        if k * _T < r_tail:
            w = w2_s[rows, :]
        else:
            w = jnp.concatenate(
                [w2_s[rows, :c_left]] + [w2t_s[c, k * _T - r_tail:(k + 1) * _T - r_tail]
                                         for c in range(kd - _W2_LEFT)], axis=1)
        acc = acc + _mm(tile(hs[k // (_NB // _T)], k % (_NB // _T)), w)
    out_s[...] = acc.astype(out_s.dtype)
    pltpu.sync_copy(out_s, o_h)


@jax.jit
def pallas_interleave_layers__sliding_block_cached__mixer_channel_mlp__decode_kernel(
    A_x: jax.Array,
    A_k_cache: jax.Array,
    A_v_cache: jax.Array,
    A_wq: jax.Array,
    A_wo: jax.Array,
    B_x: jax.Array,
    B_w1: jax.Array,
    B_b1: jax.Array,
    B_w2: jax.Array,
    B_b2: jax.Array,
):
    del B_x
    nb_, sq, d_model = A_x.shape
    _, hkv, sk, dh = A_k_cache.shape
    d_ff = B_w1.shape[1]
    win = min(4096, max(256, sk // 4))
    rep = _HQ // hkv
    assert (nb_, sq, rep, dh) == (8, 1, 8, _T)
    n_sem = 12 + d_model // _T - _W2_LEFT

    hbm = pl.BlockSpec(memory_space=pltpu.HBM)
    vmem = pltpu.VMEM
    out = pl.pallas_call(
        _kernel,
        out_shape=jax.ShapeDtypeStruct((nb_, d_model), A_x.dtype),
        in_specs=[hbm] * 9,
        out_specs=hbm,
        scratch_shapes=[
            vmem((nb_, d_model), A_x.dtype),
            vmem((nb_, hkv, win, dh), _BF),
            vmem((nb_ * hkv, dh, win), _BF),
            vmem((nb_, hkv, win, dh), _BF),
            vmem(A_wq.shape, _BF),
            vmem(A_wo.shape, _BF),
            vmem(B_w1.shape, _BF),
            vmem(B_b1.shape, B_b1.dtype),
            vmem(B_w2.shape, _BF),
            vmem((d_model // _T - _W2_LEFT, d_ff - _W2_TAIL, _T), _BF),
            vmem(B_b2.shape, B_b2.dtype),
            vmem((_HQ, nb_, dh), _F32),
            vmem((nb_, _HQ * dh), _F32),
            vmem((2, nb_, d_ff), _F32),
            vmem((nb_ * hkv, rep, win), _F32),
            vmem((nb_ * hkv, rep, dh), _F32),
            vmem((_HQ, nb_, dh), _F32),
            vmem((nb_, d_ff), _F32),
            vmem((nb_, d_model), _F32),
            vmem((nb_, d_model), A_x.dtype),
            pltpu.SMEM((_SIDE, d_model), _BF),
            pltpu.SMEM((_SIDE, d_model), _BF),
            pltpu.SemaphoreType.DMA((n_sem,)),
            pltpu.SemaphoreType.DMA((2,)),
        ],
        compiler_params=pltpu.CompilerParams(
            vmem_limit_bytes=100 * 1024 * 1024, disable_semaphore_checks=True),
    )(A_x.reshape(nb_, d_model), A_k_cache, A_v_cache, A_wq, A_wo, B_w1, B_b1, B_w2, B_b2)
    return out.reshape(nb_, sq, d_model)
```

```python
import functools
import math

import jax
import jax.numpy as jnp
from jax import lax
import jax.experimental.pallas as pl
import jax.experimental.pallas.tpu as pltpu

_BF = jnp.bfloat16
_F32 = jnp.float32
_EPS = 1e-5
_T = 128
_NB = 4 * _T
_HQ = 32
_W2_MID, _W2_TAIL = 1664, 2560
_W2_LEFT = 4
_SIDE = 176
_HOLD = 2


def _mm(a, b):
    return jnp.dot(a, b, preferred_element_type=_F32)


def _ln_stats(x):
    m = jnp.mean(x, axis=-1, keepdims=True)
    d = x - m
    v = jnp.mean(d * d, axis=-1, keepdims=True)
    return m, d, lax.rsqrt(v + _EPS)


def _gelu(x):
    c = math.sqrt(2.0 / math.pi)
    return x * (0.5 * (1.0 + jnp.tanh(c * (x + 0.044715 * (x * x * x)))))


def _swap8(vs):
    row = lax.broadcasted_iota(jnp.int32, (8, _T), 0)
    vs = list(vs)
    for s in (4, 2, 1):
        hi = (row & s) != 0
        out = [None] * 8
        for i in range(8):
            if i & s:
                continue
            a, b = vs[i], vs[i + s]
            out[i] = jnp.where(hi, pltpu.roll(b, s, 0), a)
            out[i + s] = jnp.where(hi, b, pltpu.roll(a, 8 - s, 0))
        vs = out
    return vs


def _body(x_h, k_h, v_h, wq_h, wo_h, w1_h, b1_h, w2_h, b2_h, o_h,
            x_s, k_s, kt_s, v_s, wq_s, wo_s, w1_s, b1_s, w2_s, w2t_s, b2_s,
            q_s, cq_s, c1_s, p_s, l_s, a_s, h_s, r_s, out_s, side0, side1, sems, side_sems):
    nb_, d_model = x_s.shape
    hkv, win, dh = k_s.shape[1], k_s.shape[2], k_s.shape[3]
    rep = _HQ // hkv
    d_ff = w1_s.shape[1]
    sk = k_h.shape[2]
    kd, kf = d_model // _T, d_ff // _T
    sm_c = dh ** -0.5 * math.log2(math.e)
    r_mid, r_tail, c_left = _W2_MID, _W2_TAIL, _W2_LEFT * _T
    r_half = r_mid - 4 * _SIDE
    r_side = r_half - 2 * _SIDE

    bands = [(0, r_side, 0, d_model), (r_half, r_tail, 0, c_left),
             (r_tail, d_ff, 0, c_left), (r_mid, r_tail, c_left, d_model)]
    copies = [
        (wq_h, wq_s), (x_h, x_s), (b1_h, b1_s), (b2_h, b2_s),
        (k_h.at[:, :, pl.ds(sk - win, win)], k_s),
        (v_h.at[:, :, pl.ds(sk - win, win)], v_s),
        (wo_h, wo_s), (w1_h, w1_s),
    ] + [(w2_h.at[r0:r1, c0:c1], w2_s.at[r0:r1, c0:c1]) for r0, r1, c0, c1 in bands]
    dmas = [pltpu.make_async_copy(a, b, sems.at[i]) for i, (a, b) in enumerate(copies)]
    n_fix = len(dmas) - _W2_LEFT

    def tail_dma(c):
        idx = (pl.ds(r_tail, d_ff - r_tail), pl.ds(c * _T, _T))
        return pltpu.make_async_copy(w2_h.at[idx], w2t_s.at[c - _W2_LEFT], sems.at[n_fix + c])

    def side_piece(i):
        if i % 2 == 0:
            return (pl.ds(r_side + i // 2 * _SIDE, _SIDE),)
        return pl.ds(r_half + (i - 1) * _SIDE, 2 * _SIDE), pl.ds(c_left, d_model - c_left)

    def side_in(i):
        return pltpu.make_async_copy(
            w2_h.at[side_piece(i)], (side0, side1)[i % 2], side_sems.at[i % 2])

    def side_out(i):
        return pltpu.make_async_copy(
            (side0, side1)[i % 2], w2_s.at[side_piece(i)], side_sems.at[i % 2])

    def side_forward(i):
        side_in(i).wait()
        side_out(i).start()

    def side_refill(i):
        side_out(i - 2).wait()
        side_in(i).start()

    dmas[0].start()
    side_in(0).start()
    side_in(1).start()
    for d in dmas[1:]:
        d.start()
    for c in range(_W2_LEFT, kd):
        tail_dma(c).start()
    d_wq, d_x, d_b1, d_b2, d_k, d_v, d_wo, d_w1 = dmas[:8]

    def tile(v, i):
        return v[:, i * _T:(i + 1) * _T]

    def proj(lhs, w_ref, cols):
        acc = None
        for k in range(lhs.shape[1] // _T):
            y = _mm(tile(lhs, k), w_ref[k * _T:(k + 1) * _T, cols])
            acc = y if acc is None else acc + y
        return acc

    ones = jnp.ones((nb_, d_model), _F32)

    side_forward(0)
    d_x.wait()
    x0 = x_s[...].astype(_F32)
    _, d0, r0_ = _ln_stats(x0)
    lhs = jnp.concatenate([d0 * r0_, ones], axis=0).astype(_BF)
    d_wq.wait()

    @pl.loop(0, hkv)
    def _(j):
        qs = []
        for n in range(rep * dh // _NB):
            cols = pl.ds(pl.multiple_of(j * (rep * dh) + n * _NB, _NB), _NB)
            y = proj(lhs, wq_s, cols)
            cq_s[:, cols] = y[nb_:]
            qs += [tile(y[:nb_], i) for i in range(_NB // _T)]
        for b, qb in enumerate(_swap8(qs)):
            q_s[j * nb_ + b] = qb

    side_forward(1)
    d_k.wait()

    @pl.loop(0, hkv * nb_)
    def _(g):
        pl.when(g == 8)(lambda: side_refill(2))
        pl.when(g == 22)(lambda: side_refill(3))
        kt = k_s[g % nb_, g // nb_].T
        kt_s[g] = kt
        s = _mm(q_s[g].astype(_BF), kt)
        p = jnp.exp2((s - jnp.max(s, axis=-1, keepdims=True)) * sm_c)
        l_s[g] = jnp.broadcast_to(1.0 / jnp.sum(p, axis=-1, keepdims=True), (rep, dh))
        p_s[g] = p

    d_v.wait()

    @pl.loop(0, hkv)
    def _(j):
        os_ = []
        for b in range(nb_):
            g = j * nb_ + b
            os_.append(_mm(p_s[g].astype(_BF), v_s[b, j]) * l_s[g])
        for r, o in enumerate(_swap8(os_)):
            a_s[j * rep + r] = o

    side_forward(2)
    d_wo.wait()

    def wo_body(j, acc):
        for r in range(rep):
            hd = j * rep + r
            rows = pl.ds(pl.multiple_of(hd * dh, dh), dh)
            acc = acc + _mm(a_s[hd].astype(_BF), wo_s[rows, :])
        return acc

    x1 = lax.fori_loop(0, hkv, wo_body, x0)

    _, d1, r1_ = _ln_stats(x1)
    _, d1, r1_ = _ln_stats(d1 * r1_)
    lhs = jnp.concatenate([d1 * r1_, ones], axis=0).astype(_BF)
    d_b1.wait()
    d_b2.wait()
    b2 = b2_s[...].astype(_F32).reshape(1, d_model)
    c1_s[0] = jnp.broadcast_to(b1_s[...].astype(_F32).reshape(1, d_ff), (nb_, d_ff))
    side_forward(3)
    d_w1.wait()

    @pl.loop(0, d_ff // _NB)
    def _(n):
        cols = pl.ds(pl.multiple_of(n * _NB, _NB), _NB)
        y = proj(lhs, w1_s, cols)
        c1_s[1, :, cols] = y[nb_:]
        h_s[:, cols] = _gelu(y[:nb_] + c1_s[0, :, cols])

    r_s[...] = x1 + b2

    def w2_part(r0, r1, c0, c1):
        r_s[:, c0:c1] += proj(h_s[:, r0:r1].astype(_BF), w2_s.at[r0:r1], slice(c0, c1))

    q_raw = [None] * _HQ

    n_q = _HQ * dh // _NB

    def q_update(xc, c, blocks):
        for n in blocks:
            y = _mm(xc, wq_s[c * _T:(c + 1) * _T, n * _NB:(n + 1) * _NB])
            for i in range(_NB // _T):
                hd = n * (_NB // _T) + i
                q_raw[hd] = tile(y, i) if q_raw[hd] is None else q_raw[hd] + tile(y, i)

    r_full = r_half // _T * _T
    dmas[8].wait()
    side_out(2).wait()
    w2_part(0, r_full, 0, d_model)
    dmas[9].wait()
    w2_part(r_full, r_tail, 0, c_left)
    dmas[10].wait()
    w2_part(r_tail, d_ff, 0, c_left)
    x2b = [r_s[:, c * _T:(c + 1) * _T].astype(_BF) for c in range(_W2_LEFT)]
    for c in range(_W2_LEFT):
        q_update(x2b[c], c, range(n_q - (_HOLD if c == _W2_LEFT - 1 else 0)))
    side_out(3).wait()
    w2_part(r_full, r_mid, c_left, d_model)
    dmas[11].wait()
    w2_part(r_mid, r_tail, c_left, d_model)
    h_tail = h_s[:, r_tail:].astype(_BF)
    for c in range(_W2_LEFT, kd):
        if c == kd - 1:
            seen = jnp.concatenate(x2b, axis=1).astype(_F32)
            m_seen, d_seen, _ = _ln_stats(seen)
            ss_seen = jnp.sum(d_seen * d_seen, axis=-1, keepdims=True)
        tail_dma(c).wait()
        cols = slice(c * _T, (c + 1) * _T)
        xc = r_s[:, cols] + proj(h_tail, w2t_s.at[c - _W2_LEFT], slice(None))
        r_s[:, cols] = xc
        x2b.append(xc.astype(_BF))
        q_update(x2b[c - 1], c - 1, range(n_q - _HOLD, n_q))
        q_update(x2b[c], c, range(n_q - (_HOLD if c < kd - 1 else 0)))

    x2 = r_s[...]
    e = x2b[-1].astype(_F32) - m_seen
    shift = jnp.sum(e, axis=-1, keepdims=True) * (1.0 / d_model)
    var = (ss_seen + jnp.sum(e * e, axis=-1, keepdims=True)) * (1.0 / d_model) - shift * shift
    m, rstd = m_seen + shift, lax.rsqrt(var + _EPS)
    qg = []
    for j in range(hkv):
        qs = _swap8([(q_raw[hd] - m * cq_s[:, hd * dh:(hd + 1) * dh]) * rstd
                     for hd in range(j * rep, (j + 1) * rep)])
        for b in range(0, nb_, 2):
            qg.append(jnp.concatenate(qs[b:b + 2], axis=0).astype(_BF))

    def qk(i):
        ps, ls = [], []
        for u in range(2):
            s = _mm(qg[i], kt_s[2 * i + u])[u * rep:(u + 1) * rep]
            p = jnp.exp2((s - jnp.max(s, axis=-1, keepdims=True)) * sm_c)
            ls.append(1.0 / jnp.sum(p, axis=-1, keepdims=True))
            ps.append(p)
        return jnp.concatenate(ps, axis=0).astype(_BF), ls

    def pv(i, p, ls):
        j, b = divmod(2 * i, nb_)
        return [_mm(p, v_s[b + u, j])[u * rep:(u + 1) * rep] * ls[u] for u in range(2)]

    n_pair = hkv * nb_ // 2
    ahead = 2
    pend, os_, heads = {}, [], []
    for i in range(n_pair + ahead):
        if i < n_pair:
            pend[i] = qk(i)
        if i >= ahead:
            os_ += pv(i - ahead, *pend.pop(i - ahead))
            if len(os_) == nb_:
                heads += [o.astype(_BF) for o in _swap8(os_)]
                os_ = []

    x3 = []
    for n in range(d_model // _NB):
        acc = x2[:, n * _NB:(n + 1) * _NB]
        for hd in range(_HQ):
            acc = acc + _mm(heads[hd], wo_s[hd * dh:(hd + 1) * dh, n * _NB:(n + 1) * _NB])
        x3.append(acc)
    x3b = [v.astype(_BF) for v in x3]
    x3 = jnp.concatenate(x3, axis=1)

    m1, d3, r3 = _ln_stats(jnp.concatenate(x3b, axis=1).astype(_F32))
    m2, _, r4 = _ln_stats(d3 * r3)
    sa = r3 * r4
    sb = (m1 * r3 + m2) * r4

    def w1_part(n, half, acc):
        for k in range(_NB // _T):
            kk = half * (_NB // _T) + k
            y = _mm(tile(x3b[half], k), w1_s[kk * _T:(kk + 1) * _T, n * _NB:(n + 1) * _NB])
            acc = y if acc is None else acc + y
        return acc

    lead = 2
    part = [w1_part(n, 0, None) for n in range(lead)]
    hs = []
    for n in range(d_ff // _NB):
        y = w1_part(n, 1, part[n] if n < lead else w1_part(n, 0, None))
        cols = slice(n * _NB, (n + 1) * _NB)
        hs.append(_gelu(y * sa - sb * c1_s[1, :, cols] + c1_s[0, :, cols]).astype(_BF))

    acc = x3 + b2
    for k in range(kf):
        rows = slice(k * _T, (k + 1) * _T)
        if k * _T < r_tail:
            w = w2_s[rows, :]
        else:
            w = jnp.concatenate(
                [w2_s[rows, :c_left]] + [w2t_s[c, k * _T - r_tail:(k + 1) * _T - r_tail]
                                         for c in range(kd - _W2_LEFT)], axis=1)
        acc = acc + _mm(tile(hs[k // (_NB // _T)], k % (_NB // _T)), w)
    out_s[...] = acc.astype(out_s.dtype)
    pltpu.sync_copy(out_s, o_h)


def _kernel(*refs):
    n_main = 12 + refs[0].shape[1] // _T - _W2_LEFT
    pl.run_scoped(functools.partial(_body, *refs),
                  pltpu.SemaphoreType.DMA((n_main,)), pltpu.SemaphoreType.DMA((2,)))


@jax.jit
def pallas_interleave_layers__sliding_block_cached__mixer_channel_mlp__decode_kernel(
    A_x: jax.Array,
    A_k_cache: jax.Array,
    A_v_cache: jax.Array,
    A_wq: jax.Array,
    A_wo: jax.Array,
    B_x: jax.Array,
    B_w1: jax.Array,
    B_b1: jax.Array,
    B_w2: jax.Array,
    B_b2: jax.Array,
):
    del B_x
    nb_, sq, d_model = A_x.shape
    _, hkv, sk, dh = A_k_cache.shape
    d_ff = B_w1.shape[1]
    win = min(4096, max(256, sk // 4))
    rep = _HQ // hkv
    assert (nb_, sq, rep, dh) == (8, 1, 8, _T)

    hbm = pl.BlockSpec(memory_space=pltpu.HBM)
    vmem = pltpu.VMEM
    out = pl.pallas_call(
        _kernel,
        out_shape=jax.ShapeDtypeStruct((nb_, d_model), A_x.dtype),
        in_specs=[hbm] * 9,
        out_specs=hbm,
        scratch_shapes=[
            vmem((nb_, d_model), A_x.dtype),
            vmem((nb_, hkv, win, dh), _BF),
            vmem((nb_ * hkv, dh, win), _BF),
            vmem((nb_, hkv, win, dh), _BF),
            vmem(A_wq.shape, _BF),
            vmem(A_wo.shape, _BF),
            vmem(B_w1.shape, _BF),
            vmem(B_b1.shape, B_b1.dtype),
            vmem(B_w2.shape, _BF),
            vmem((d_model // _T - _W2_LEFT, d_ff - _W2_TAIL, _T), _BF),
            vmem(B_b2.shape, B_b2.dtype),
            vmem((_HQ, nb_, dh), _F32),
            vmem((nb_, _HQ * dh), _F32),
            vmem((2, nb_, d_ff), _F32),
            vmem((nb_ * hkv, rep, win), _F32),
            vmem((nb_ * hkv, rep, dh), _F32),
            vmem((_HQ, nb_, dh), _F32),
            vmem((nb_, d_ff), _F32),
            vmem((nb_, d_model), _F32),
            vmem((nb_, d_model), A_x.dtype),
            pltpu.SMEM((_SIDE, d_model), _BF),
            pltpu.SMEM((2 * _SIDE, d_model - _W2_LEFT * _T), _BF),
        ],
        compiler_params=pltpu.CompilerParams(vmem_limit_bytes=80 * 1024 * 1024),
    )(A_x.reshape(nb_, d_model), A_k_cache, A_v_cache, A_wq, A_wo, B_w1, B_b1, B_w2, B_b2)
    return out.reshape(nb_, sq, d_model)
```

```python
import functools
import math

import jax
import jax.numpy as jnp
from jax import lax
import jax.experimental.pallas as pl
import jax.experimental.pallas.tpu as pltpu

_BF = jnp.bfloat16
_F32 = jnp.float32
_EPS = 1e-5
_T = 128
_NB = 4 * _T
_HQ = 32
_W2_MID, _W2_TAIL = 1536, 2560
_W2_LEFT = 4
_SIDE = 176
_HOLD = 2


def _mm(a, b):
    return jnp.dot(a, b, preferred_element_type=_F32)


def _ln_stats(x):
    m = jnp.mean(x, axis=-1, keepdims=True)
    d = x - m
    v = jnp.mean(d * d, axis=-1, keepdims=True)
    return m, d, lax.rsqrt(v + _EPS)


def _gelu(x):
    c = math.sqrt(2.0 / math.pi)
    return x * (0.5 * (1.0 + jnp.tanh(c * (x + 0.044715 * (x * x * x)))))


def _swap8(vs):
    row = lax.broadcasted_iota(jnp.int32, (8, _T), 0)
    vs = list(vs)
    for s in (4, 2, 1):
        hi = (row & s) != 0
        out = [None] * 8
        for i in range(8):
            if i & s:
                continue
            a, b = vs[i], vs[i + s]
            out[i] = jnp.where(hi, pltpu.roll(b, s, 0), a)
            out[i + s] = jnp.where(hi, b, pltpu.roll(a, 8 - s, 0))
        vs = out
    return vs


def _body(x_h, k_h, v_h, wq_h, wo_h, w1_h, b1_h, w2_h, b2_h, o_h,
          x_s, k_s, kt_s, v_s, wq_s, wo_s, w1_s, b1_s, w2_s, w2t_s, b2_s,
          q_s, cq_s, c1_s, p_s, l_s, a_s, h_s, r_s, out_s, side0, side1, sems, side_sems):
    nb_, d_model = x_s.shape
    hkv, win, dh = k_s.shape[1], k_s.shape[2], k_s.shape[3]
    rep = _HQ // hkv
    d_ff = w1_s.shape[1]
    sk = k_h.shape[2]
    kd, kf = d_model // _T, d_ff // _T
    sm_c = dh ** -0.5 * math.log2(math.e)
    r_mid, r_tail, c_left = _W2_MID, _W2_TAIL, _W2_LEFT * _T
    r_half = r_mid - 4 * _SIDE
    r_side = r_half - 2 * _SIDE

    bands = [(0, r_side, 0, d_model), (r_half, r_tail, 0, c_left),
             (r_tail, d_ff, 0, c_left), (r_mid, r_tail, c_left, d_model)]
    copies = [
        (wq_h, wq_s), (x_h, x_s), (b1_h, b1_s), (b2_h, b2_s),
        (k_h.at[:, :, pl.ds(sk - win, win)], k_s),
        (v_h.at[:, :, pl.ds(sk - win, win)], v_s),
        (wo_h, wo_s), (w1_h, w1_s),
    ] + [(w2_h.at[r0:r1, c0:c1], w2_s.at[r0:r1, c0:c1]) for r0, r1, c0, c1 in bands]
    dmas = [pltpu.make_async_copy(a, b, sems.at[i]) for i, (a, b) in enumerate(copies)]
    n_fix = len(dmas) - _W2_LEFT

    def tail_dma(c):
        idx = (pl.ds(r_tail, d_ff - r_tail), pl.ds(c * _T, _T))
        return pltpu.make_async_copy(w2_h.at[idx], w2t_s.at[c - _W2_LEFT], sems.at[n_fix + c])

    def side_piece(i):
        if i % 2 == 0:
            return (pl.ds(r_side + i // 2 * _SIDE, _SIDE),)
        return pl.ds(r_half + (i - 1) * _SIDE, 2 * _SIDE), pl.ds(c_left, d_model - c_left)

    def side_in(i):
        return pltpu.make_async_copy(
            w2_h.at[side_piece(i)], (side0, side1)[i % 2], side_sems.at[i % 2])

    def side_out(i):
        return pltpu.make_async_copy(
            (side0, side1)[i % 2], w2_s.at[side_piece(i)], side_sems.at[i % 2])

    def side_forward(i):
        side_in(i).wait()
        side_out(i).start()

    def side_refill(i):
        side_out(i - 2).wait()
        side_in(i).start()

    dmas[0].start()
    side_in(0).start()
    side_in(1).start()
    for d in dmas[1:]:
        d.start()
    for c in range(_W2_LEFT, kd):
        tail_dma(c).start()
    d_wq, d_x, d_b1, d_b2, d_k, d_v, d_wo, d_w1 = dmas[:8]

    def tile(v, i):
        return v[:, i * _T:(i + 1) * _T]

    def proj(lhs, w_ref, cols):
        acc = None
        for k in range(lhs.shape[1] // _T):
            y = _mm(tile(lhs, k), w_ref[k * _T:(k + 1) * _T, cols])
            acc = y if acc is None else acc + y
        return acc

    ones = jnp.ones((nb_, d_model), _F32)

    side_forward(0)
    d_x.wait()
    x0 = x_s[...].astype(_F32)
    _, d0, r0_ = _ln_stats(x0)
    lhs = jnp.concatenate([d0 * r0_, ones], axis=0).astype(_BF)
    d_wq.wait()

    @pl.loop(0, hkv)
    def _(j):
        qs = []
        for n in range(rep * dh // _NB):
            cols = pl.ds(pl.multiple_of(j * (rep * dh) + n * _NB, _NB), _NB)
            y = proj(lhs, wq_s, cols)
            cq_s[:, cols] = y[nb_:]
            qs += [tile(y[:nb_], i) for i in range(_NB // _T)]
        for b, qb in enumerate(_swap8(qs)):
            q_s[j * nb_ + b] = qb

    side_forward(1)
    d_k.wait()

    @pl.loop(0, hkv * nb_)
    def _(g):
        pl.when(g == 8)(lambda: side_refill(2))
        pl.when(g == 22)(lambda: side_refill(3))
        kt = k_s[g % nb_, g // nb_].T
        kt_s[g] = kt
        s = _mm(q_s[g].astype(_BF), kt)
        p = jnp.exp2((s - jnp.max(s, axis=-1, keepdims=True)) * sm_c)
        l_s[g] = jnp.broadcast_to(1.0 / jnp.sum(p, axis=-1, keepdims=True), (rep, dh))
        p_s[g] = p

    d_v.wait()

    @pl.loop(0, hkv)
    def _(j):
        os_ = []
        for b in range(nb_):
            g = j * nb_ + b
            os_.append(_mm(p_s[g].astype(_BF), v_s[b, j]) * l_s[g])
        for r, o in enumerate(_swap8(os_)):
            a_s[j * rep + r] = o

    side_forward(2)
    d_wo.wait()

    def wo_body(j, acc):
        for r in range(rep):
            hd = j * rep + r
            rows = pl.ds(pl.multiple_of(hd * dh, dh), dh)
            acc = acc + _mm(a_s[hd].astype(_BF), wo_s[rows, :])
        return acc

    x1 = lax.fori_loop(0, hkv, wo_body, x0)

    _, d1, r1_ = _ln_stats(x1)
    _, d1, r1_ = _ln_stats(d1 * r1_)
    lhs = jnp.concatenate([d1 * r1_, ones], axis=0).astype(_BF)
    d_b1.wait()
    d_b2.wait()
    b2 = b2_s[...].astype(_F32).reshape(1, d_model)
    c1_s[0] = jnp.broadcast_to(b1_s[...].astype(_F32).reshape(1, d_ff), (nb_, d_ff))
    side_forward(3)
    d_w1.wait()

    @pl.loop(0, d_ff // _NB)
    def _(n):
        cols = pl.ds(pl.multiple_of(n * _NB, _NB), _NB)
        y = proj(lhs, w1_s, cols)
        c1_s[1, :, cols] = y[nb_:]
        h_s[:, cols] = _gelu(y[:nb_] + c1_s[0, :, cols])

    r_s[...] = x1 + b2

    def w2_part(r0, r1, c0, c1):
        r_s[:, c0:c1] += proj(h_s[:, r0:r1].astype(_BF), w2_s.at[r0:r1], slice(c0, c1))

    q_raw = [None] * _HQ
    n_q = _HQ * dh // _NB

    def q_update(xc, c, blocks):
        for n in blocks:
            y = _mm(xc, wq_s[c * _T:(c + 1) * _T, n * _NB:(n + 1) * _NB])
            for i in range(_NB // _T):
                hd = n * (_NB // _T) + i
                q_raw[hd] = tile(y, i) if q_raw[hd] is None else q_raw[hd] + tile(y, i)

    r_full = r_half // _T * _T
    dmas[8].wait()
    side_out(2).wait()
    w2_part(0, r_full, 0, d_model)
    dmas[9].wait()
    w2_part(r_full, r_tail, 0, c_left)
    dmas[10].wait()
    w2_part(r_tail, d_ff, 0, c_left)
    x2b = [r_s[:, c * _T:(c + 1) * _T].astype(_BF) for c in range(_W2_LEFT)]
    for c in range(_W2_LEFT):
        q_update(x2b[c], c, range(n_q - (_HOLD if c == _W2_LEFT - 1 else 0)))
    side_out(3).wait()
    w2_part(r_full, r_mid, c_left, d_model)
    dmas[11].wait()
    w2_part(r_mid, r_tail, c_left, d_model)
    h_tail = h_s[:, r_tail:].astype(_BF)
    for c in range(_W2_LEFT, kd):
        if c == kd - 1:
            seen = jnp.concatenate(x2b, axis=1).astype(_F32)
            m_seen, d_seen, _ = _ln_stats(seen)
            ss_seen = jnp.sum(d_seen * d_seen, axis=-1, keepdims=True)
        tail_dma(c).wait()
        cols = slice(c * _T, (c + 1) * _T)
        xc = r_s[:, cols] + proj(h_tail, w2t_s.at[c - _W2_LEFT], slice(None))
        r_s[:, cols] = xc
        x2b.append(xc.astype(_BF))
        q_update(x2b[c - 1], c - 1, range(n_q - _HOLD, n_q))
        q_update(x2b[c], c, range(n_q - (_HOLD if c < kd - 1 else 0)))

    x2 = r_s[...]
    e = x2b[-1].astype(_F32) - m_seen
    shift = jnp.sum(e, axis=-1, keepdims=True) * (1.0 / d_model)
    var = (ss_seen + jnp.sum(e * e, axis=-1, keepdims=True)) * (1.0 / d_model) - shift * shift
    m, rstd = m_seen + shift, lax.rsqrt(var + _EPS)
    qg = []
    for j in range(hkv):
        qs = _swap8([(q_raw[hd] - m * cq_s[:, hd * dh:(hd + 1) * dh]) * rstd
                     for hd in range(j * rep, (j + 1) * rep)])
        for b in range(0, nb_, 2):
            qg.append(jnp.concatenate(qs[b:b + 2], axis=0).astype(_BF))

    def qk(i):
        ps, ls = [], []
        for u in range(2):
            s = _mm(qg[i], kt_s[2 * i + u])[u * rep:(u + 1) * rep]
            p = jnp.exp2((s - jnp.max(s, axis=-1, keepdims=True)) * sm_c)
            ls.append(1.0 / jnp.sum(p, axis=-1, keepdims=True))
            ps.append(p)
        return jnp.concatenate(ps, axis=0).astype(_BF), ls

    def pv(i, p, ls):
        j, b = divmod(2 * i, nb_)
        return [_mm(p, v_s[b + u, j])[u * rep:(u + 1) * rep] * ls[u] for u in range(2)]

    n_pair = hkv * nb_ // 2
    ahead = 2
    pend, os_, heads = {}, [], []
    for i in range(n_pair + ahead):
        if i < n_pair:
            pend[i] = qk(i)
        if i >= ahead:
            os_ += pv(i - ahead, *pend.pop(i - ahead))
            if len(os_) == nb_:
                heads += [o.astype(_BF) for o in _swap8(os_)]
                os_ = []

    x3 = []
    for n in range(d_model // _NB):
        acc = x2[:, n * _NB:(n + 1) * _NB]
        for hd in range(_HQ):
            acc = acc + _mm(heads[hd], wo_s[hd * dh:(hd + 1) * dh, n * _NB:(n + 1) * _NB])
        x3.append(acc)
    x3b = [v.astype(_BF) for v in x3]
    x3 = jnp.concatenate(x3, axis=1)

    m1, d3, r3 = _ln_stats(jnp.concatenate(x3b, axis=1).astype(_F32))
    m2, _, r4 = _ln_stats(d3 * r3)
    sa = r3 * r4
    sb = (m1 * r3 + m2) * r4

    def w1_part(n, half, acc):
        for k in range(_NB // _T):
            kk = half * (_NB // _T) + k
            y = _mm(tile(x3b[half], k), w1_s[kk * _T:(kk + 1) * _T, n * _NB:(n + 1) * _NB])
            acc = y if acc is None else acc + y
        return acc

    lead = 2
    part = [w1_part(n, 0, None) for n in range(lead)]
    hs = []
    for n in range(d_ff // _NB):
        y = w1_part(n, 1, part[n] if n < lead else w1_part(n, 0, None))
        cols = slice(n * _NB, (n + 1) * _NB)
        hs.append(_gelu(y * sa - sb * c1_s[1, :, cols] + c1_s[0, :, cols]).astype(_BF))

    acc = x3 + b2
    for k in range(kf):
        rows = slice(k * _T, (k + 1) * _T)
        if k * _T < r_tail:
            w = w2_s[rows, :]
        else:
            w = jnp.concatenate(
                [w2_s[rows, :c_left]] + [w2t_s[c, k * _T - r_tail:(k + 1) * _T - r_tail]
                                         for c in range(kd - _W2_LEFT)], axis=1)
        acc = acc + _mm(tile(hs[k // (_NB // _T)], k % (_NB // _T)), w)
    out_s[...] = acc.astype(out_s.dtype)
    pltpu.sync_copy(out_s, o_h)


def _kernel(*refs):
    n_main = 12 + refs[0].shape[1] // _T - _W2_LEFT
    pl.run_scoped(functools.partial(_body, *refs),
                  pltpu.SemaphoreType.DMA((n_main,)), pltpu.SemaphoreType.DMA((2,)))


@jax.jit
def pallas_interleave_layers__sliding_block_cached__mixer_channel_mlp__decode_kernel(
    A_x: jax.Array,
    A_k_cache: jax.Array,
    A_v_cache: jax.Array,
    A_wq: jax.Array,
    A_wo: jax.Array,
    B_x: jax.Array,
    B_w1: jax.Array,
    B_b1: jax.Array,
    B_w2: jax.Array,
    B_b2: jax.Array,
):
    del B_x
    nb_, sq, d_model = A_x.shape
    _, hkv, sk, dh = A_k_cache.shape
    d_ff = B_w1.shape[1]
    win = min(4096, max(256, sk // 4))
    rep = _HQ // hkv
    assert (nb_, sq, hkv, rep, dh, d_model) == (8, 1, 4, 8, _T, 2 * _NB)
    assert d_ff % _NB == 0 and d_ff > _W2_TAIL

    hbm = pl.BlockSpec(memory_space=pltpu.HBM)
    vmem = pltpu.VMEM
    out = pl.pallas_call(
        _kernel,
        out_shape=jax.ShapeDtypeStruct((nb_, d_model), A_x.dtype),
        in_specs=[hbm] * 9,
        out_specs=hbm,
        scratch_shapes=[
            vmem((nb_, d_model), A_x.dtype),
            vmem((nb_, hkv, win, dh), _BF),
            vmem((nb_ * hkv, dh, win), _BF),
            vmem((nb_, hkv, win, dh), _BF),
            vmem(A_wq.shape, _BF),
            vmem(A_wo.shape, _BF),
            vmem(B_w1.shape, _BF),
            vmem(B_b1.shape, B_b1.dtype),
            vmem(B_w2.shape, _BF),
            vmem((d_model // _T - _W2_LEFT, d_ff - _W2_TAIL, _T), _BF),
            vmem(B_b2.shape, B_b2.dtype),
            vmem((_HQ, nb_, dh), _F32),
            vmem((nb_, _HQ * dh), _F32),
            vmem((2, nb_, d_ff), _F32),
            vmem((nb_ * hkv, rep, win), _F32),
            vmem((nb_ * hkv, rep, dh), _F32),
            vmem((_HQ, nb_, dh), _F32),
            vmem((nb_, d_ff), _F32),
            vmem((nb_, d_model), _F32),
            vmem((nb_, d_model), A_x.dtype),
            pltpu.SMEM((_SIDE, d_model), _BF),
            pltpu.SMEM((2 * _SIDE, d_model - _W2_LEFT * _T), _BF),
        ],
        compiler_params=pltpu.CompilerParams(vmem_limit_bytes=80 * 1024 * 1024),
    )(A_x.reshape(nb_, d_model), A_k_cache, A_v_cache, A_wq, A_wo, B_w1, B_b1, B_w2, B_b2)
    return out.reshape(nb_, sq, d_model)
```
